```python
import os as _os
_os.environ.setdefault("JAX_PLATFORMS", "cpu")
import jax
import jax.numpy as jnp

def _softmax(x, axis=-1):
    return jax.nn.softmax(x, axis=axis)
def _gelu(x):
    return jax.nn.gelu(x, approximate=True)
def _silu(x):
    return jax.nn.silu(x)
def _sigmoid(x):
    return jax.nn.sigmoid(x)
def _layernorm(x, axis=-1, eps=1e-5):
    m = jnp.mean(x, axis=axis, keepdims=True)
    v = jnp.var(x, axis=axis, keepdims=True)
    return (x - m) / jnp.sqrt(v + eps)
def _scatter_add(tgt, idx, src, axis=0):
    return tgt.at[idx].add(src)
def _segment_sum(src, seg, n):
    return jax.ops.segment_sum(src, seg, n)
class _Rng:
    def __init__(self, key):
        self._k = key
    def _next(self):
        self._k, sub = jax.random.split(self._k)
        return sub
    def normal(self, shape):
        return jax.random.normal(self._next(), shape, dtype=jnp.bfloat16)
    def randint(self, lo, hi, shape):
        return jax.random.randint(self._next(), shape, lo, hi, dtype=jnp.int32)
    def uniform(self, shape, lo=0.0, hi=1.0):
        return jax.random.uniform(self._next(), shape, jnp.bfloat16, lo, hi)
    def permutation(self, n):
        return jax.random.permutation(self._next(), n)


kernel_name = 'standalone__dcn_v2_cross__recsys'

def setup_inputs():
    _rng = _Rng(jax.random.key(int.from_bytes(__import__("os").urandom(4), "little")))
    _w = (lambda a: (lambda t: t.astype(jnp.bfloat16) if jnp.issubdtype(t.dtype, jnp.floating) else t)(jnp.asarray(a)))
    B, F, D, L = 4096, 26, 128, 6
    Din = min(F * D, 1024)
    return {
        "x0": _w((lambda *s: _rng.normal(s) * 0.05)(B, Din)),
        "ws": _w((lambda *s: _rng.normal(s) * 0.05)(L, Din, Din)),
        "bs": _w((lambda *s: _rng.normal(s) * 0.05)(L, Din)),
    }

def reference(x0, ws, bs):
    x = x0
    for l in range(ws.shape[0]):
        x = x0 * (x @ ws[l] + bs[l]) + x
    return x
```

```python
import jax
import jax.numpy as jnp
import jax.experimental.pallas as pl
import jax.experimental.pallas.tpu as pltpu

R = 128
SB = True
OORD = (2, 4, 0, 3, 6, 1, 5)
IORD = (2, 4, 0, 3, 1, 6, 5)
f32 = jnp.float32
bf16 = jnp.bfloat16
u32 = jnp.uint32

A_T = [((0,1),(3,1)), ((2,1),(3,1)), ((0,1),), ((3,1),), ((0,1),(1,1)), ((2,1),(0,-1)), ((1,1),(3,-1))]
B_T = [((0,1),(3,1)), ((0,1),), ((1,1),(3,-1)), ((2,1),(0,-1)), ((3,1),), ((0,1),(1,1)), ((2,1),(3,1))]
C_T = [((0,1),(3,1),(4,-1),(6,1)), ((2,1),(4,1)), ((1,1),(3,1)), ((0,1),(1,-1),(2,1),(5,1))]

def lin(terms, get):
    acc = None
    for i, s in terms:
        v = get(i)
        acc = v if acc is None else (acc + v if s > 0 else acc - v)
    return acc

def rc(qo, qi):
    return 2 * (qo >> 1) + (qi >> 1), 2 * (qo & 1) + (qi & 1)

def fin(q, order):
    return max((p for p, _ in C_T[q]), key=order.index)

def kept(p, order):
    return any(p in [t for t, _ in C_T[q]] and fin(q, order) != p for q in range(4))

def _kernel(x0_ref, ws_hbm, bs_ref, o_ref, sems, bf_ref, raw, wp, *sc):
    L = ws_hbm.shape[0]
    pid = pl.program_id(0)
    zs, zl = pid >> 10, pid >> 11

    def wcopy(l):
        return pltpu.make_async_copy(ws_hbm.at[l], raw.at[l], sems.at[l])

    xs, x0s, mi, do, sb = sc[0:32], sc[32:48], sc[48:62], sc[62:90], sc[90:94]

    def blk(qo, qi):
        rb, cb = rc(qo, qi)
        return slice(rb * R, rb * R + R), slice(cb * 256, cb * 256 + 256)

    def layer(l, par, getx, getw, putx):
        for no, o in enumerate(OORD):
            mm = mi[7 * ((par + no) % 2):]
            for i in IORD:
                a = lin(A_T[i], lambda qi: lin(A_T[o], lambda qo: getx(qo * 4 + qi))).astype(bf16)
                m = jnp.dot(a, getw(o, i), preferred_element_type=f32)
                if kept(i, IORD):
                    mm[i][zs] = m
                for qi in range(4):
                    if fin(qi, IORD) != i: continue
                    d = lin(C_T[qi], lambda j: m if j == i else mm[j][zl])
                    if kept(o, OORD):
                        do[o * 4 + qi][zs] = d
                    for qo in range(4):
                        if fin(qo, OORD) != o: continue
                        c = lin(C_T[qo], lambda j: d if j == o else do[j * 4 + qi][zl])
                        k = qo * 4 + qi
                        putx(k, x0s[k][zl] * (c + bf_ref[l, 0:1, blk(qo, qi)[1]]) + getx(k))

    def put_out(k, v):
        o_ref[blk(k // 4, k % 4)] = v.astype(bf16)

    @pl.when(pid == 0)
    def _():
        wcopy(0).start()
        bv = bs_ref[...].astype(f32)
        for l in range(L):
            bf_ref[l] = jnp.broadcast_to(bv[l:l+1], (8, bv.shape[1]))
        for k in range(16):
            v = x0_ref[blk(k // 4, k % 4)].astype(f32)
            x0s[k][zs] = v
            xs[k][zs] = v
        def body(l, c):
            wcopy(l).wait()
            pl.when(l + 1 < L)(lambda: wcopy(l + 1).start())
            have = set()
            def raww(qo, qi):
                rb, cb = rc(qo, qi)
                return raw[l, rb * 256:(rb + 1) * 256, cb * 256:(cb + 1) * 256].astype(f32)
            def gets(o, qi):
                if len(B_T[o]) == 1 or not SB:
                    return lin(B_T[o], lambda qo: raww(qo, qi))
                if (o, qi) in have:
                    return sb[qi][zl]
                have.add((o, qi))
                v = lin(B_T[o], lambda qo: raww(qo, qi))
                sb[qi][zs] = v
                return v
            def getw(o, i):
                w = lin(B_T[i], lambda qi: gets(o, qi)).astype(bf16)
                wp[l, o * 7 + i] = pltpu.bitcast(w, u32)
                return w
            def putx(k, v):
                xs[k][1 - (l & 1)] = v
                put_out(k, v)
            layer(l, 0, lambda k: xs[k][l & 1], getw, putx)
            return c
        jax.lax.fori_loop(0, L, body, 0)

    @pl.when(pid != 0)
    def _():
        seen = set()
        for l in range(L):
            def getx(k):
                if l > 0:
                    return xs[16 * (l % 2) + k][zl]
                if k in seen:
                    return x0s[k][zl]
                seen.add(k)
                v = x0_ref[blk(k // 4, k % 4)].astype(f32)
                x0s[k][zs] = v
                return v
            def putx(k, v):
                xs[16 * (1 - l % 2) + k][zs] = v
            layer(l, l, getx, lambda o, i: pltpu.bitcast(wp[l, o * 7 + i], bf16), put_out if l == L - 1 else putx)

@jax.jit
def pallas_standalone__dcn_v2_cross__recsys_kernel(x0, ws, bs):
    B, D = x0.shape
    L = ws.shape[0]
    BM = 4 * R
    return pl.pallas_call(
        _kernel,
        grid=(B // BM,),
        in_specs=[pl.BlockSpec((BM, D), lambda i: (i, 0)),
                  pl.BlockSpec(memory_space=pl.ANY),
                  pl.BlockSpec((L, D), lambda i: (0, 0))],
        out_specs=pl.BlockSpec((BM, D), lambda i: (i, 0)),
        out_shape=jax.ShapeDtypeStruct((B, D), x0.dtype),
        scratch_shapes=[pltpu.SemaphoreType.DMA((L,)), pltpu.VMEM((L, 8, D), f32)]
            + [pltpu.VMEM((L, D, D), bf16), pltpu.VMEM((L, 49, 128, 256), u32)]
            + [pltpu.VMEM((2, R, 256), f32)] * 16 + [pltpu.VMEM((1, R, 256), f32)] * 74
            + [pltpu.VMEM((1, 256, 256), f32)] * 4,
        compiler_params=pltpu.CompilerParams(dimension_semantics=("arbitrary",), vmem_limit_bytes=110*1024*1024),
    )(x0, ws, bs)
```
